```python
import jax
import jax.numpy as jnp

def _softmax(x, axis=-1):
    return jax.nn.softmax(x, axis=axis)
def _gelu(x):
    return jax.nn.gelu(x, approximate=True)
def _silu(x):
    return jax.nn.silu(x)
def _sigmoid(x):
    return jax.nn.sigmoid(x)
def _layernorm(x, axis=-1, eps=1e-5):
    m = jnp.mean(x, axis=axis, keepdims=True)
    v = jnp.var(x, axis=axis, keepdims=True)
    return (x - m) / jnp.sqrt(v + eps)
def _scatter_add(tgt, idx, src, axis=0):
    return tgt.at[idx].add(src)
def _segment_sum(src, seg, n):
    return jax.ops.segment_sum(src, seg, n)
class _Rng:
    def __init__(self, key):
        self._k = key
    def _next(self):
        self._k, sub = jax.random.split(self._k)
        return sub
    def normal(self, shape):
        return jax.random.normal(self._next(), shape, dtype=jnp.bfloat16)
    def randint(self, lo, hi, shape):
        return jax.random.randint(self._next(), shape, lo, hi, dtype=jnp.int32)
    def uniform(self, shape, lo=0.0, hi=1.0):
        return jax.random.uniform(self._next(), shape, jnp.bfloat16, lo, hi)
    def permutation(self, n):
        return jax.random.permutation(self._next(), n)


kernel_name = 'recurrent_scan__mha_block_cached__moe_arch_mod__decode'

def setup_inputs():
    _rng = _Rng(jax.random.key(int.from_bytes(__import__("os").urandom(4), "little")))
    _w = (lambda a: (lambda t: t.astype(jnp.bfloat16) if jnp.issubdtype(t.dtype, jnp.floating) else t)(jnp.asarray(a)))
    def _A_setup():
        B, Sq, D = 2, 1, 512
        H, Sk, Dh = 32, 16384, 128
        return {
            "x": _w((lambda *s: _rng.normal(s) * 0.05)(B, Sq, D)),
            "k_cache": _w((lambda *s: _rng.normal(s) * 0.05)(B, H, Sk, Dh)),
            "v_cache": _w((lambda *s: _rng.normal(s) * 0.05)(B, H, Sk, Dh)),
            "wq": _w((lambda *s: _rng.normal(s) * 0.05)(D, H * Dh) * (D ** -0.5)),
            "wo": _w((lambda *s: _rng.normal(s) * 0.05)(H * Dh, D) * ((H * Dh) ** -0.5)),
        }
    _A_in = _A_setup()

    def _B_setup():
        B, S, D, F, C = 2, 1, 512, 1792, 1
        return {
            "x": _w((lambda *s: _rng.normal(s) * 0.05)(B, S, D)),
            "w_r": _w((lambda *s: _rng.normal(s) * 0.05)(D)),
            "w_gate": _w((lambda *s: _rng.normal(s) * 0.05)(D, F)),
            "w_up": _w((lambda *s: _rng.normal(s) * 0.05)(D, F)),
            "w_down": _w((lambda *s: _rng.normal(s) * 0.05)(F, D)),
        }
    _B_in = _B_setup()

    return {
        "A_x": _A_in["x"],
        "A_k_cache": _A_in["k_cache"],
        "A_v_cache": _A_in["v_cache"],
        "A_wq": _A_in["wq"],
        "A_wo": _A_in["wo"],
        "B_x": _B_in["x"],
        "B_w_r": _B_in["w_r"],
        "B_w_gate": _B_in["w_gate"],
        "B_w_up": _B_in["w_up"],
        "B_w_down": _B_in["w_down"],
    }

def reference(A_x, A_k_cache, A_v_cache, A_wq, A_wo, B_x, B_w_r, B_w_gate, B_w_up, B_w_down):
    def _A_ref(x, k_cache, v_cache, wq, wo):
        B, Sq, D = x.shape
        H, Dh = 32, 128
        q = (lambda x, *d: x.transpose(*d))((x @ wq).reshape(B, Sq, H, Dh), 0, 2, 1, 3)
        scores = jnp.einsum("bhqd,bhkd->bhqk", q, k_cache) * (Dh ** -0.5)
        p = _softmax(scores, axis=-1)
        o = jnp.einsum("bhqk,bhkd->bhqd", p, v_cache)
        return (lambda x, *d: x.transpose(*d))(o, 0, 2, 1, 3).reshape(B, Sq, H * Dh) @ wo

    def _B_ref(x, w_r, w_gate, w_up, w_down):
        B, S, D = x.shape
        C = 1
        r = x @ w_r
        idx = jnp.argsort(-r, axis=-1)[:, :C]
        idx_e = jnp.repeat(idx.reshape(B, C, 1), D, axis=2)
        x_sel = jnp.take_along_axis(x, idx_e, axis=1)
        g = _silu(x_sel @ w_gate)
        u = x_sel @ w_up
        y = (g * u) @ w_down
        r_sel = _sigmoid(jnp.take_along_axis(r, idx, axis=1))
        y = y * r_sel.reshape(B, C, 1)
        b_off = (jnp.arange(B) * S).reshape(B, 1)
        flat_idx = (idx + b_off).reshape(B * C)
        zero = (x * 0.0).reshape(B * S, D)
        upd = _scatter_add(zero, flat_idx, y.reshape(B * C, D), axis=0)
        return x + upd.reshape(B, S, D)

    x = A_x
    xn = _layernorm(x, axis=-1)
    s = _A_ref(xn, A_k_cache, A_v_cache, A_wq, A_wo)
    g = _silu(_B_ref(xn, B_w_r, B_w_gate, B_w_up, B_w_down))
    return x + s * g
```

```python
import functools

import jax
import jax.numpy as jnp
from jax import lax
import jax.experimental.pallas as pl
import jax.experimental.pallas.tpu as pltpu

_ROWS = 8
_PIECE = 128
_F32 = jnp.float32
_BF16 = jnp.bfloat16
_NT = (((1,), (1,)), ((), ()))


def _dot(a, b):
    return jnp.dot(a, b, preferred_element_type=_F32)


def _kernel(
    x_hbm, k_hbm, v_hbm, wq_hbm, wo_hbm, wr_hbm, wg_hbm, wu_hbm, wd_hbm,
    o_hbm,
    kbuf, vbuf, x_vm, wq_vm, wo_vm, wr_vm, wg_vm, wu_vm, wd_vm, sc_vm, o_vm,
    ksem, vsem, wsem,
    *, nb, nh, sk, chunk, nbuf,
):
    dh = kbuf.shape[-1]
    d = x_vm.shape[-1]
    cph = sk // chunk
    nheads = nb * nh
    nchunks = nheads * cph
    npiece = chunk // _PIECE
    scale = dh ** -0.5

    def piece(src, dst, sem, c, slot, j):
        row = pl.multiple_of(c * chunk + j * _PIECE, _PIECE)
        return pltpu.make_async_copy(
            src.at[pl.ds(row, _PIECE)],
            dst.at[slot, pl.ds(j * _PIECE, _PIECE)],
            sem.at[slot])

    def start_k(t):
        for j in range(npiece):
            piece(k_hbm, kbuf, ksem, t, t % nbuf, j).start(priority=j % 2)

    def start_v(t):
        for j in range(npiece):
            piece(v_hbm, vbuf, vsem, t - cph, t % nbuf, j).start(priority=j % 2)

    def start_kv(t):
        for j in range(npiece):
            piece(k_hbm, kbuf, ksem, t, t % nbuf, j).start(priority=0)
            piece(v_hbm, vbuf, vsem, t - cph, t % nbuf, j).start(priority=1)

    def start_step(t):
        pl.when(t < cph)(lambda: start_k(t))
        pl.when(jnp.logical_and(t >= cph, t < nchunks))(lambda: start_kv(t))
        pl.when(jnp.logical_and(t >= nchunks, t < nchunks + cph))(lambda: start_v(t))

    def wait(buf, sem, slot):
        pltpu.make_async_copy(buf.at[slot], buf.at[slot], sem.at[slot]).wait()

    pairs = ((x_hbm, x_vm), (wr_hbm, wr_vm), (wq_hbm, wq_vm), (wg_hbm, wg_vm),
             (wu_hbm, wu_vm), (wd_hbm, wd_vm), (wo_hbm, wo_vm))
    wcopy = [pltpu.make_async_copy(s, t, wsem.at[i]) for i, (s, t) in enumerate(pairs)]
    for c in wcopy:
        c.start()

    @pl.loop(0, nbuf)
    def _(t):
        start_step(t)

    row = lax.broadcasted_iota(jnp.int32, (_ROWS, d), 0) % nb
    wcopy[0].wait()
    x_in = x_vm[...].astype(_F32)
    x = jnp.broadcast_to(x_in[0:1], (_ROWS, d))
    for b in range(1, nb):
        x = jnp.where(row == b, x_in[b:b + 1], x)
    xc = x - jnp.mean(x, axis=-1, keepdims=True)
    var = jnp.mean(xc * xc, axis=-1, keepdims=True)
    xn_b = (xc / jnp.sqrt(var + 1e-5)).astype(_BF16)
    xn = xn_b.astype(_F32)

    wcopy[1].wait()
    w_r = wr_vm[...].astype(_F32)
    r = sum(xn[:, j * 128:(j + 1) * 128] * w_r[j:j + 1] for j in range(d // 128))
    r = jnp.sum(r, axis=-1, keepdims=True)
    wcopy[3].wait()
    gate = _dot(xn_b, wg_vm[...])
    wcopy[4].wait()
    up = _dot(xn_b, wu_vm[...])
    wcopy[5].wait()
    y = _dot((jax.nn.silu(gate) * up).astype(_BF16), wd_vm[...])
    g = jax.nn.silu(xn + (xn * 0.0 + y * jax.nn.sigmoid(r)))
    wcopy[2].wait()
    wcopy[6].wait()

    def q_of(n):
        col = pl.multiple_of((n % nh) * dh, dh)
        return _dot(xn_b, wq_vm[:, pl.ds(col, dh)]).astype(_BF16)

    def fold(a, op):
        out = a[:, :128]
        for j in range(1, a.shape[1] // 128):
            out = op(out, a[:, j * 128:(j + 1) * 128])
        return out

    def qk(t, c, q, mx):
        s = lax.dot_general(q, kbuf[t % nbuf], _NT, preferred_element_type=_F32)
        sc_vm[c] = s
        return jnp.maximum(mx, fold(s, jnp.maximum))

    def pv(t, c, m, l, acc):
        p = jnp.exp((sc_vm[c] - m) * scale)
        return l + fold(p, jnp.add), acc + _dot(p.astype(_BF16), vbuf[t % nbuf])

    def project(n, l, acc, out):
        o = (acc / jnp.sum(l, axis=-1, keepdims=True)).astype(_BF16)
        w = wo_vm[pl.ds(pl.multiple_of((n % nh) * dh, dh), dh), :]
        return out + jnp.where(row == n // nh, _dot(o, w), 0.0)

    neg = jnp.full((_ROWS, 128), -jnp.inf, _F32)
    zero = jnp.zeros((_ROWS, 128), _F32)

    q = q_of(0)

    def first(c, mx):
        wait(kbuf, ksem, c % nbuf)
        mx = qk(c, c, q, mx)
        start_step(c + nbuf)
        return mx

    mx = lax.fori_loop(0, cph, first, neg)

    def head(n, carry):
        m, out = carry
        q = q_of(n)

        def step(c, carry):
            mx, l, acc = carry
            t = n * cph + c
            wait(kbuf, ksem, t % nbuf)
            wait(vbuf, vsem, t % nbuf)
            l, acc = pv(t, c, m, l, acc)
            mx = qk(t, c, q, mx)
            start_step(t + nbuf)
            return mx, l, acc

        mx, l, acc = lax.fori_loop(0, cph, step, (neg, zero, zero))
        return jnp.max(mx, axis=-1, keepdims=True), project(n - 1, l, acc, out)

    m, out = lax.fori_loop(
        1, nheads, head,
        (jnp.max(mx, axis=-1, keepdims=True), jnp.zeros((_ROWS, d), _F32)))

    def last(c, carry):
        t = nchunks + c
        wait(vbuf, vsem, t % nbuf)
        carry = pv(t, c, m, *carry)
        start_step(t + nbuf)
        return carry

    l, acc = lax.fori_loop(0, cph, last, (zero, zero))
    out = project(nheads - 1, l, acc, out)

    o_vm[...] = (x + out * g)[:nb].astype(o_vm.dtype)
    pltpu.sync_copy(o_vm, o_hbm)


def _build(chunk=2048, nbuf=6, **params):
    def call(A_x, A_k_cache, A_v_cache, A_wq, A_wo, B_x, B_w_r, B_w_gate, B_w_up, B_w_down):
        del B_x
        nb, nh, sk, dh = A_k_cache.shape
        d = A_x.shape[-1]
        vm = lambda a: pltpu.VMEM(a.shape, a.dtype)
        x = A_x.reshape(nb, d)
        w_r = B_w_r.reshape(d // 128, 128)
        ring = pltpu.VMEM((nbuf, chunk, dh), A_k_cache.dtype)
        hbm = pl.BlockSpec(memory_space=pltpu.HBM)
        return pl.pallas_call(
            functools.partial(_kernel, nb=nb, nh=nh, sk=sk, chunk=chunk, nbuf=nbuf),
            in_specs=[hbm] * 9,
            out_specs=hbm,
            out_shape=jax.ShapeDtypeStruct(x.shape, x.dtype),
            scratch_shapes=[
                ring, ring, vm(x), vm(A_wq), vm(A_wo), vm(w_r),
                vm(B_w_gate), vm(B_w_up), vm(B_w_down),
                pltpu.VMEM((sk // chunk, _ROWS, chunk), _F32), vm(x),
                pltpu.SemaphoreType.DMA((nbuf,)), pltpu.SemaphoreType.DMA((nbuf,)),
                pltpu.SemaphoreType.DMA((7,)),
            ],
            compiler_params=pltpu.CompilerParams(vmem_limit_bytes=64 * 2**20, **params),
        )(x, A_k_cache.reshape(nb * nh * sk, dh), A_v_cache.reshape(nb * nh * sk, dh),
          A_wq, A_wo, w_r, B_w_gate, B_w_up, B_w_down).reshape(A_x.shape)

    return call


@jax.jit
def pallas_recurrent_scan__mha_block_cached__moe_arch_mod__decode_kernel(
    A_x: jax.Array,
    A_k_cache: jax.Array,
    A_v_cache: jax.Array,
    A_wq: jax.Array,
    A_wo: jax.Array,
    B_x: jax.Array,
    B_w_r: jax.Array,
    B_w_gate: jax.Array,
    B_w_up: jax.Array,
    B_w_down: jax.Array,
):
    return _build()(A_x, A_k_cache, A_v_cache, A_wq, A_wo, B_x, B_w_r, B_w_gate, B_w_up, B_w_down)
```

```python
import functools

import jax
import jax.numpy as jnp
from jax import lax
import jax.experimental.pallas as pl
import jax.experimental.pallas.tpu as pltpu

_ROWS = 8
_PIECE = 128
_F32 = jnp.float32
_BF16 = jnp.bfloat16
_NT = (((1,), (1,)), ((), ()))


def _dot(a, b):
    return jnp.dot(a, b, preferred_element_type=_F32)


def _kernel(
    x_hbm, k_hbm, v_hbm, wq_hbm, wo_hbm, wr_hbm, wg_hbm, wu_hbm, wd_hbm,
    o_hbm,
    kbuf, vbuf, x_vm, wq_vm, wo_vm, wr_vm, wg_vm, wu_vm, wd_vm, sc_vm, o_vm,
    ksem, vsem, wsem,
    *, nb, nh, sk, chunk, nbuf,
):
    dh = kbuf.shape[-1]
    d = x_vm.shape[-1]
    cph = sk // chunk
    nheads = nb * nh
    nchunks = nheads * cph
    npiece = chunk // _PIECE
    scale = dh ** -0.5

    def piece(src, dst, sem, c, slot, j):
        ntop = src.shape[1]
        return pltpu.make_async_copy(
            src.at[c // cph, j % ntop, :, (c % cph) * (npiece // ntop) + j // ntop],
            dst.at[slot, j],
            sem.at[slot])

    def landed(buf, t):
        return buf[t % nbuf].reshape(chunk, dh)

    def start_k(t):
        for j in range(npiece):
            piece(k_hbm, kbuf, ksem, t, t % nbuf, j).start(priority=j % 2)

    def start_v(t):
        for j in range(npiece):
            piece(v_hbm, vbuf, vsem, t - cph, t % nbuf, j).start(priority=j % 2)

    def start_kv(t):
        for j in range(npiece):
            piece(k_hbm, kbuf, ksem, t, t % nbuf, j).start(priority=0)
            piece(v_hbm, vbuf, vsem, t - cph, t % nbuf, j).start(priority=1)

    def start_step(t):
        pl.when(t < cph)(lambda: start_k(t))
        pl.when(jnp.logical_and(t >= cph, t < nchunks))(lambda: start_kv(t))
        pl.when(jnp.logical_and(t >= nchunks, t < nchunks + cph))(lambda: start_v(t))

    def wait(buf, sem, slot):
        pltpu.make_async_copy(buf.at[slot], buf.at[slot], sem.at[slot]).wait()

    pairs = ((x_hbm, x_vm), (wr_hbm, wr_vm), (wq_hbm, wq_vm), (wg_hbm, wg_vm),
             (wu_hbm, wu_vm), (wd_hbm, wd_vm), (wo_hbm, wo_vm))
    wcopy = [pltpu.make_async_copy(s, t, wsem.at[i]) for i, (s, t) in enumerate(pairs)]
    for c in wcopy:
        c.start()

    @pl.loop(0, nbuf)
    def _(t):
        start_step(t)

    row = lax.broadcasted_iota(jnp.int32, (_ROWS, d), 0) % nb
    wcopy[0].wait()
    x_in = x_vm[...].astype(_F32)
    x = jnp.broadcast_to(x_in[0:1], (_ROWS, d))
    for b in range(1, nb):
        x = jnp.where(row == b, x_in[b:b + 1], x)
    xc = x - jnp.mean(x, axis=-1, keepdims=True)
    var = jnp.mean(xc * xc, axis=-1, keepdims=True)
    xn_b = (xc / jnp.sqrt(var + 1e-5)).astype(_BF16)
    xn = xn_b.astype(_F32)

    wcopy[1].wait()
    w_r = wr_vm[...].astype(_F32)
    r = sum(xn[:, j * 128:(j + 1) * 128] * w_r[j:j + 1] for j in range(d // 128))
    r = jnp.sum(r, axis=-1, keepdims=True)
    wcopy[3].wait()
    gate = _dot(xn_b, wg_vm[...])
    wcopy[4].wait()
    up = _dot(xn_b, wu_vm[...])
    wcopy[5].wait()
    y = _dot((jax.nn.silu(gate) * up).astype(_BF16), wd_vm[...])
    g = jax.nn.silu(xn + (xn * 0.0 + y * jax.nn.sigmoid(r)))
    wcopy[2].wait()
    wcopy[6].wait()

    def q_of(n):
        col = pl.multiple_of((n % nh) * dh, dh)
        return _dot(xn_b, wq_vm[:, pl.ds(col, dh)]).astype(_BF16)

    def fold(a, op):
        out = a[:, :128]
        for j in range(1, a.shape[1] // 128):
            out = op(out, a[:, j * 128:(j + 1) * 128])
        return out

    def qk(t, c, q, mx):
        s = lax.dot_general(q, landed(kbuf, t), _NT, preferred_element_type=_F32)
        sc_vm[c] = s
        return jnp.maximum(mx, fold(s, jnp.maximum))

    def pv(t, c, m, l, acc):
        p = jnp.exp((sc_vm[c] - m) * scale)
        return l + fold(p, jnp.add), acc + _dot(p.astype(_BF16), landed(vbuf, t))

    def project(n, l, acc, out):
        o = (acc / jnp.sum(l, axis=-1, keepdims=True)).astype(_BF16)
        w = wo_vm[pl.ds(pl.multiple_of((n % nh) * dh, dh), dh), :]
        return out + jnp.where(row == n // nh, _dot(o, w), 0.0)

    neg = jnp.full((_ROWS, 128), -jnp.inf, _F32)
    zero = jnp.zeros((_ROWS, 128), _F32)

    q = q_of(0)

    def first(c, mx):
        wait(kbuf, ksem, c % nbuf)
        mx = qk(c, c, q, mx)
        start_step(c + nbuf)
        return mx

    mx = lax.fori_loop(0, cph, first, neg)

    def head(n, carry):
        m, out = carry
        q = q_of(n)

        def step(c, carry):
            mx, l, acc = carry
            t = n * cph + c
            wait(kbuf, ksem, t % nbuf)
            wait(vbuf, vsem, t % nbuf)
            l, acc = pv(t, c, m, l, acc)
            mx = qk(t, c, q, mx)
            start_step(t + nbuf)
            return mx, l, acc

        mx, l, acc = lax.fori_loop(0, cph, step, (neg, zero, zero))
        return jnp.max(mx, axis=-1, keepdims=True), project(n - 1, l, acc, out)

    m, out = lax.fori_loop(
        1, nheads, head,
        (jnp.max(mx, axis=-1, keepdims=True), jnp.zeros((_ROWS, d), _F32)))

    def last(c, carry):
        t = nchunks + c
        wait(vbuf, vsem, t % nbuf)
        carry = pv(t, c, m, *carry)
        start_step(t + nbuf)
        return carry

    l, acc = lax.fori_loop(0, cph, last, (zero, zero))
    out = project(nheads - 1, l, acc, out)

    o_vm[...] = (x + out * g)[:nb].astype(o_vm.dtype)
    pltpu.sync_copy(o_vm, o_hbm)


def _build(chunk=2048, nbuf=6, sub=32, ntop=2, **params):
    def call(A_x, A_k_cache, A_v_cache, A_wq, A_wo, B_x, B_w_r, B_w_gate, B_w_up, B_w_down):
        del B_x
        nb, nh, sk, dh = A_k_cache.shape
        d = A_x.shape[-1]
        vm = lambda a: pltpu.VMEM(a.shape, a.dtype)
        x = A_x.reshape(nb, d)
        w_r = B_w_r.reshape(d // 128, 128)
        cnt = _PIECE // sub
        view = (nb * nh, ntop, cnt, sk // (ntop * _PIECE), sub, dh)
        ring = pltpu.VMEM((nbuf, chunk // _PIECE, cnt, sub, dh), A_k_cache.dtype)
        hbm = pl.BlockSpec(memory_space=pltpu.HBM)
        return pl.pallas_call(
            functools.partial(_kernel, nb=nb, nh=nh, sk=sk, chunk=chunk, nbuf=nbuf),
            in_specs=[hbm] * 9,
            out_specs=hbm,
            out_shape=jax.ShapeDtypeStruct(x.shape, x.dtype),
            scratch_shapes=[
                ring, ring, vm(x), vm(A_wq), vm(A_wo), vm(w_r),
                vm(B_w_gate), vm(B_w_up), vm(B_w_down),
                pltpu.VMEM((sk // chunk, _ROWS, chunk), _F32), vm(x),
                pltpu.SemaphoreType.DMA((nbuf,)), pltpu.SemaphoreType.DMA((nbuf,)),
                pltpu.SemaphoreType.DMA((7,)),
            ],
            compiler_params=pltpu.CompilerParams(vmem_limit_bytes=64 * 2**20, **params),
        )(x, A_k_cache.reshape(view), A_v_cache.reshape(view),
          A_wq, A_wo, w_r, B_w_gate, B_w_up, B_w_down).reshape(A_x.shape)

    return call


@jax.jit
def pallas_recurrent_scan__mha_block_cached__moe_arch_mod__decode_kernel(
    A_x: jax.Array,
    A_k_cache: jax.Array,
    A_v_cache: jax.Array,
    A_wq: jax.Array,
    A_wo: jax.Array,
    B_x: jax.Array,
    B_w_r: jax.Array,
    B_w_gate: jax.Array,
    B_w_up: jax.Array,
    B_w_down: jax.Array,
):
    return _build()(A_x, A_k_cache, A_v_cache, A_wq, A_wo, B_x, B_w_r, B_w_gate, B_w_up, B_w_down)
```

```python
import functools

import jax
import jax.numpy as jnp
from jax import lax
import jax.experimental.pallas as pl
import jax.experimental.pallas.tpu as pltpu

_ROWS = 8
_SUB = 32
_RUNS = 4
_TOP = 2
_F32 = jnp.float32
_BF16 = jnp.bfloat16
_NT = (((1,), (1,)), ((), ()))


def _dot(a, b):
    return jnp.dot(a, b, preferred_element_type=_F32)


def _mat(a):
    return a.reshape(-1, a.shape[-1])


def _fold(a, op):
    out = a[:, :128]
    for j in range(1, a.shape[1] // 128):
        out = op(out, a[:, j * 128:(j + 1) * 128])
    return out


def _wait_all(buf, sem):
    pltpu.make_async_copy(buf, buf, sem).wait()


def _body(
    ring_sem, w_sem, *,
    x_hbm, k_hbm, v_hbm, wq_hbm, wo_hbm, wr_hbm, wg_hbm, wu_hbm, wd_hbm,
    kbuf, vbuf, x_vm, wq_vm, wo_vm, wr_vm, wg_vm, wu_vm, wd_vm, sc_vm, o_vm,
    out_copy,
):
    nb, d = x_vm.shape
    nbuf, npiece = kbuf.shape[:2]
    dh = kbuf.shape[-1]
    nheads = k_hbm.shape[0]
    nh = nheads // nb
    cph = sc_vm.shape[0]
    nchunks = nheads * cph
    scale = dh ** -0.5

    def piece(src, dst, c, slot, j):
        return pltpu.make_async_copy(
            src.at[c // cph, j % _TOP, :, (c % cph) * (npiece // _TOP) + j // _TOP],
            dst.at[slot, j],
            ring_sem.at[slot])

    def start_step(t):
        slot = t % nbuf

        @pl.when(t < cph)
        def _():
            for j in range(npiece):
                piece(k_hbm, kbuf, t, slot, j).start(priority=j % 2)

        @pl.when(jnp.logical_and(t >= cph, t < nchunks))
        def _():
            for j in range(npiece):
                piece(k_hbm, kbuf, t, slot, j).start(priority=0)
                piece(v_hbm, vbuf, t - cph, slot, j).start(priority=1)

        @pl.when(jnp.logical_and(t >= nchunks, t < nchunks + cph))
        def _():
            for j in range(npiece):
                piece(v_hbm, vbuf, t - cph, slot, j).start(priority=j % 2)

    def start(src, dst, sem, idx, queue):
        pltpu.make_async_copy(src.at[idx], dst.at[idx], w_sem.at[sem]).start(priority=queue)

    def rows(i, n):
        return pl.ds(pl.multiple_of(i * n, n), n)

    x_copy = pltpu.make_async_copy(x_hbm, x_vm, w_sem.at[0])
    wr_copy = pltpu.make_async_copy(wr_hbm, wr_vm, w_sem.at[1])
    ncol = wq_vm.shape[-1] // 512
    every = slice(None)

    @pl.loop(0, wq_vm.shape[2] // 8)
    def _(i):
        for j in range(2 * ncol):
            start(wq_hbm, wq_vm, 2, (j % 2, every, rows(i, 8), pl.ds(j // 2 * 512, 512)), j % 2)

    x_copy.start()
    wr_copy.start(priority=1)
    half = wg_vm.shape[-1] // 2

    @pl.loop(0, wg_vm.shape[1] // 8)
    def _(i):
        for j in range(2):
            start(wg_hbm, wg_vm, 3, (every, rows(i, 8), pl.ds(j * half, half)), 0)
            start(wu_hbm, wu_vm, 4, (every, rows(i, 8), pl.ds(j * half, half)), 1)

    @pl.loop(0, wd_vm.shape[2] // 8)
    def _(i):
        for j in range(2):
            start(wd_hbm, wd_vm, 5, (every, j, rows(i, 8)), j)

    @pl.loop(0, wo_vm.shape[2] // 8)
    def _(i):
        for j in range(2):
            start(wo_hbm, wo_vm, 6, (j, every, rows(i, 8)), j)

    pl.loop(0, nbuf)(start_step)

    row = lax.broadcasted_iota(jnp.int32, (_ROWS, d), 0) % nb
    x_copy.wait()
    x_in = x_vm[...].astype(_F32)
    x = jnp.broadcast_to(x_in[0:1], (_ROWS, d))
    for b in range(1, nb):
        x = jnp.where(row == b, x_in[b:b + 1], x)
    xc = x - jnp.mean(x, axis=-1, keepdims=True)
    var = jnp.mean(xc * xc, axis=-1, keepdims=True)
    xn_b = (xc / jnp.sqrt(var + 1e-5)).astype(_BF16)
    xn = xn_b.astype(_F32)

    wr_copy.wait()
    w_r = wr_vm[...].astype(_F32)
    r = sum(xn[:, j * 128:(j + 1) * 128] * w_r[j:j + 1] for j in range(d // 128))
    r = jnp.sum(r, axis=-1, keepdims=True)
    _wait_all(wg_vm, w_sem.at[3])
    _wait_all(wu_vm, w_sem.at[4])
    _wait_all(wd_vm, w_sem.at[5])
    gate = _dot(xn_b, _mat(wg_vm[...]))
    up = _dot(xn_b, _mat(wu_vm[...]))
    y = _dot((jax.nn.silu(gate) * up).astype(_BF16), _mat(wd_vm[...]))
    g = jax.nn.silu(xn + (xn * 0.0 + y * jax.nn.sigmoid(r)))
    _wait_all(wq_vm, w_sem.at[2])
    _wait_all(wo_vm, w_sem.at[6])

    def q_of(n):
        return _dot(xn_b, _mat(wq_vm[:, :, :, rows(n % nh, dh)])).astype(_BF16)

    def qk(slot, c, q, mx):
        s = lax.dot_general(q, _mat(kbuf[slot]), _NT, preferred_element_type=_F32)
        sc_vm[c] = s
        return jnp.maximum(mx, _fold(s, jnp.maximum))

    def pv(slot, c, m, l, acc):
        p = jnp.exp((sc_vm[c] - m) * scale)
        return l + _fold(p, jnp.add), acc + _dot(p.astype(_BF16), _mat(vbuf[slot]))

    def project(n, l, acc, out):
        o = (acc / jnp.sum(l, axis=-1, keepdims=True)).astype(_BF16)
        hps = wo_vm.shape[2] // dh
        seg = n % nh // hps
        w = wo_vm[seg // _RUNS, seg % _RUNS, rows(n % hps, dh), :]
        return out + jnp.where(row == n // nh, _dot(o, w), 0.0)

    neg = jnp.full((_ROWS, 128), -jnp.inf, _F32)
    zero = jnp.zeros((_ROWS, 128), _F32)
    q0 = q_of(0)

    def first(c, mx):
        slot = c % nbuf
        _wait_all(kbuf.at[slot], ring_sem.at[slot])
        mx = qk(slot, c, q0, mx)
        start_step(c + nbuf)
        return mx

    def head(n, carry):
        m, out = carry
        q = q_of(n)

        def step(c, carry):
            mx, l, acc = carry
            t = n * cph + c
            slot = t % nbuf
            _wait_all(kbuf.at[slot], ring_sem.at[slot])
            _wait_all(vbuf.at[slot], ring_sem.at[slot])
            l, acc = pv(slot, c, m, l, acc)
            mx = qk(slot, c, q, mx)
            start_step(t + nbuf)
            return mx, l, acc

        mx, l, acc = lax.fori_loop(0, cph, step, (neg, zero, zero))
        return jnp.max(mx, axis=-1, keepdims=True), project(n - 1, l, acc, out)

    m = jnp.max(lax.fori_loop(0, cph, first, neg), axis=-1, keepdims=True)
    m, out = lax.fori_loop(1, nheads, head, (m, jnp.zeros((_ROWS, d), _F32)))

    def last(c, carry):
        t = nchunks + c
        slot = t % nbuf
        _wait_all(vbuf.at[slot], ring_sem.at[slot])
        carry = pv(slot, c, m, *carry)
        start_step(t + nbuf)
        return carry

    l, acc = lax.fori_loop(0, cph, last, (zero, zero))
    out = project(nheads - 1, l, acc, out)
    o_vm[...] = (x + out * g)[:nb].astype(o_vm.dtype)
    out_copy.start()


def _kernel(
    x_hbm, k_hbm, v_hbm, wq_hbm, wo_hbm, wr_hbm, wg_hbm, wu_hbm, wd_hbm,
    o_hbm,
    kbuf, vbuf, x_vm, wq_vm, wo_vm, wr_vm, wg_vm, wu_vm, wd_vm, sc_vm, o_vm, o_sem,
):
    out_copy = pltpu.make_async_copy(o_vm, o_hbm, o_sem)
    pl.run_scoped(
        functools.partial(
            _body, x_hbm=x_hbm, k_hbm=k_hbm, v_hbm=v_hbm, wq_hbm=wq_hbm, wo_hbm=wo_hbm,
            wr_hbm=wr_hbm, wg_hbm=wg_hbm, wu_hbm=wu_hbm, wd_hbm=wd_hbm,
            kbuf=kbuf, vbuf=vbuf, x_vm=x_vm, wq_vm=wq_vm, wo_vm=wo_vm, wr_vm=wr_vm,
            wg_vm=wg_vm, wu_vm=wu_vm, wd_vm=wd_vm, sc_vm=sc_vm, o_vm=o_vm,
            out_copy=out_copy),
        pltpu.SemaphoreType.DMA((kbuf.shape[0],)),
        pltpu.SemaphoreType.DMA((7,)))
    out_copy.wait()


def _build(chunk=2048, nbuf=6, **params):
    def call(A_x, A_k_cache, A_v_cache, A_wq, A_wo, B_x, B_w_r, B_w_gate, B_w_up, B_w_down):
        del B_x
        nb, nh, sk, dh = A_k_cache.shape
        d = A_x.shape[-1]
        split = lambda a, *lead: a.reshape(*lead, -1, a.shape[-1])
        heads = (nb * nh, _TOP, _RUNS, -1, _SUB, dh)
        x = A_x.reshape(nb, d)
        weights = (split(A_wq, 2, _RUNS), split(A_wo, 2, _RUNS), B_w_r.reshape(-1, 128),
                   split(B_w_gate, 2), split(B_w_up, 2), split(B_w_down, _RUNS, 2))
        vm = lambda a: pltpu.VMEM(a.shape, a.dtype)
        ring = pltpu.VMEM((nbuf, chunk // (_RUNS * _SUB), _RUNS, _SUB, dh), A_k_cache.dtype)
        hbm = pl.BlockSpec(memory_space=pltpu.HBM)
        return pl.pallas_call(
            _kernel,
            in_specs=[hbm] * 9,
            out_specs=hbm,
            out_shape=jax.ShapeDtypeStruct(x.shape, x.dtype),
            scratch_shapes=[
                ring, ring, vm(x), *map(vm, weights),
                pltpu.VMEM((sk // chunk, _ROWS, chunk), _F32), vm(x),
                pltpu.SemaphoreType.DMA(()),
            ],
            compiler_params=pltpu.CompilerParams(vmem_limit_bytes=64 * 2**20, **params),
        )(x, A_k_cache.reshape(heads), A_v_cache.reshape(heads), *weights).reshape(A_x.shape)

    return call


@jax.jit
def pallas_recurrent_scan__mha_block_cached__moe_arch_mod__decode_kernel(
    A_x: jax.Array,
    A_k_cache: jax.Array,
    A_v_cache: jax.Array,
    A_wq: jax.Array,
    A_wo: jax.Array,
    B_x: jax.Array,
    B_w_r: jax.Array,
    B_w_gate: jax.Array,
    B_w_up: jax.Array,
    B_w_down: jax.Array,
):
    return _build()(A_x, A_k_cache, A_v_cache, A_wq, A_wo, B_x, B_w_r, B_w_gate, B_w_up, B_w_down)
```

```python
import functools

import jax
import jax.numpy as jnp
from jax import lax
import jax.experimental.pallas as pl
import jax.experimental.pallas.tpu as pltpu

_ROWS = 8
_SUB = 64
_RUNS = 2
_TOP = 2
_PAIR = 2
_WRUNS = 4
_F32 = jnp.float32
_BF16 = jnp.bfloat16
_NT = (((1,), (1,)), ((), ()))


def _dot(a, b):
    return jnp.dot(a, b, preferred_element_type=_F32)


def _mat(a):
    return a.reshape(-1, a.shape[-1])


def _fold(a, op):
    out = a[:, :128]
    for j in range(1, a.shape[1] // 128):
        out = op(out, a[:, j * 128:(j + 1) * 128])
    return out


def _block(i, n):
    return pl.ds(pl.multiple_of(i * n, n), n)


def _wait_all(buf, sem):
    pltpu.make_async_copy(buf, buf, sem).wait()


def _body(hbm, vmem, out_copy, ring_sem, w_sem):
    x_hbm, k_hbm, v_hbm, wq_hbm, wo_hbm, wr_hbm, wg_hbm, wu_hbm, wd_hbm = hbm
    ring, x_vm, wq_vm, wo_vm, wr_vm, wg_vm, wu_vm, wd_vm, sc_vm, o_vm = vmem
    nb, d = x_vm.shape
    nbuf, depth, dh = ring.shape[0], ring.shape[3], ring.shape[-1]
    npairs = k_hbm.shape[0]
    nh = npairs * _PAIR // nb
    cpp = sc_vm.shape[0]
    nchunks = npairs * cpp
    scale = dh ** -0.5

    def start_step(t):
        slot = t % nbuf

        def start_piece(kv, j, queue):
            src, c = (k_hbm, t) if kv == 0 else (v_hbm, t - cpp)
            top, i, z = j % _TOP, j // _TOP % _PAIR, j // (_TOP * _PAIR)
            pltpu.make_async_copy(
                src.at[c // cpp, i, :, top, (c % cpp) * depth + z],
                ring.at[slot, kv, i, z, top],
                ring_sem.at[slot]).start(priority=queue)

        pieces = range(depth * _PAIR * _TOP)

        @pl.when(t < cpp)
        def _():
            for j in pieces:
                start_piece(0, j, j % 2)

        @pl.when(jnp.logical_and(t >= cpp, t < nchunks))
        def _():
            for j in pieces:
                start_piece(0, j, 0)
                start_piece(1, j, 1)

        @pl.when(jnp.logical_and(t >= nchunks, t < nchunks + cpp))
        def _():
            for j in pieces:
                start_piece(1, j, j % 2)

    def start(src, dst, sem, idx, queue):
        pltpu.make_async_copy(src.at[idx], dst.at[idx], w_sem.at[sem]).start(priority=queue)

    every = slice(None)

    @pl.loop(0, wq_vm.shape[2] // 8)
    def _(i):
        for j in range(2 * wq_vm.shape[-1] // 512):
            start(wq_hbm, wq_vm, 0, (j % 2, every, _block(i, 8), pl.ds(j // 2 * 512, 512)), j % 2)

    start(x_hbm, x_vm, 1, every, 0)
    start(wr_hbm, wr_vm, 2, every, 1)

    @pl.loop(0, wg_vm.shape[1] // 8)
    def _(i):
        half = wg_vm.shape[-1] // 2
        for j in range(2):
            start(wg_hbm, wg_vm, 3, (every, _block(i, 8), pl.ds(j * half, half)), 0)
            start(wu_hbm, wu_vm, 4, (every, _block(i, 8), pl.ds(j * half, half)), 1)

    @pl.loop(0, wd_vm.shape[2] // 8)
    def _(i):
        for j in range(2):
            start(wd_hbm, wd_vm, 5, (every, j, _block(i, 8)), j)

    @pl.loop(0, wo_vm.shape[2] // 8)
    def _(i):
        for j in range(2):
            start(wo_hbm, wo_vm, 6, (j, every, _block(i, 8)), j)

    pl.loop(0, nbuf)(start_step)
    for i, buf in enumerate((wq_vm, x_vm, wr_vm, wg_vm, wu_vm, wd_vm, wo_vm)):
        _wait_all(buf, w_sem.at[i])

    row = lax.broadcasted_iota(jnp.int32, (_ROWS, d), 0) % nb
    x_in = x_vm[...].astype(_F32)
    x = jnp.broadcast_to(x_in[0:1], (_ROWS, d))
    for b in range(1, nb):
        x = jnp.where(row == b, x_in[b:b + 1], x)
    xc = x - jnp.mean(x, axis=-1, keepdims=True)
    var = jnp.mean(xc * xc, axis=-1, keepdims=True)
    xn_b = (xc / jnp.sqrt(var + 1e-5)).astype(_BF16)
    xn = xn_b.astype(_F32)

    w_r = wr_vm[...].astype(_F32)
    r = sum(xn[:, j * 128:(j + 1) * 128] * w_r[j:j + 1] for j in range(d // 128))
    r = jnp.sum(r, axis=-1, keepdims=True)
    gate = _dot(xn_b, _mat(wg_vm[...]))
    up = _dot(xn_b, _mat(wu_vm[...]))
    y = _dot((jax.nn.silu(gate) * up).astype(_BF16), _mat(wd_vm[...]))
    g = jax.nn.silu(xn + (xn * 0.0 + y * jax.nn.sigmoid(r)))

    pair = range(_PAIR)

    def q_of(u):
        cols = _block(u * _PAIR % nh // _PAIR, _PAIR * dh)
        q = _dot(xn_b, _mat(wq_vm[:, :, :, cols])).astype(_BF16)
        return [q[:, i * dh:(i + 1) * dh] for i in pair]

    def qk(slot, c, q, mx):
        s = [lax.dot_general(q[i], _mat(ring[slot, 0, i]), _NT, preferred_element_type=_F32)
             for i in pair]
        for i in pair:
            sc_vm[c, i] = s[i]
        return [jnp.maximum(mx[i], _fold(s[i], jnp.maximum)) for i in pair]

    def pv(slot, c, m, l, acc):
        p = [jnp.exp((sc_vm[c, i] - m[i]) * scale) for i in pair]
        return ([l[i] + _fold(p[i], jnp.add) for i in pair],
                [acc[i] + _dot(p[i].astype(_BF16), _mat(ring[slot, 1, i])) for i in pair])

    def row_max(mx):
        return [jnp.max(a, axis=-1, keepdims=True) for a in mx]

    def project(u, l, acc, out):
        o = jnp.concatenate(
            [acc[i] / jnp.sum(l[i], axis=-1, keepdims=True) for i in pair], axis=-1)
        per_run = wo_vm.shape[2] // (_PAIR * dh)
        hp = u * _PAIR % nh // _PAIR
        seg = hp // per_run
        w = wo_vm[seg // _WRUNS, seg % _WRUNS, _block(hp % per_run, _PAIR * dh), :]
        return out + jnp.where(row == u * _PAIR // nh, _dot(o.astype(_BF16), w), 0.0)

    neg = [jnp.full((_ROWS, 128), -jnp.inf, _F32)] * _PAIR
    zero = [jnp.zeros((_ROWS, 128), _F32)] * _PAIR
    q0 = q_of(0)

    def first(t, mx):
        slot = t % nbuf
        _wait_all(ring.at[slot, 0], ring_sem.at[slot])
        mx = qk(slot, t, q0, mx)
        start_step(t + nbuf)
        return mx

    def middle(u, carry):
        m, out = carry
        q = q_of(u)

        def step(c, carry):
            mx, l, acc = carry
            t = u * cpp + c
            slot = t % nbuf
            _wait_all(ring.at[slot], ring_sem.at[slot])
            l, acc = pv(slot, c, m, l, acc)
            mx = qk(slot, c, q, mx)
            start_step(t + nbuf)
            return mx, l, acc

        mx, l, acc = lax.fori_loop(0, cpp, step, (neg, zero, zero))
        return row_max(mx), project(u - 1, l, acc, out)

    m = row_max(lax.fori_loop(0, cpp, first, neg))
    m, out = lax.fori_loop(1, npairs, middle, (m, jnp.zeros((_ROWS, d), _F32)))

    def last(c, carry, refill=True):
        t = nchunks + c
        slot = t % nbuf
        _wait_all(ring.at[slot, 1], ring_sem.at[slot])
        carry = pv(slot, c, m, *carry)
        if refill:
            start_step(t + nbuf)
        return carry

    l, acc = last(cpp - 1, lax.fori_loop(0, cpp - 1, last, (zero, zero)), refill=False)
    out = project(npairs - 1, l, acc, out)
    o_vm[...] = (x + out * g)[:nb].astype(o_vm.dtype)
    out_copy.start()


def _kernel(*refs):
    hbm, o_hbm, vmem, o_sem = refs[:9], refs[9], refs[10:-1], refs[-1]
    out_copy = pltpu.make_async_copy(vmem[-1], o_hbm, o_sem)
    pl.run_scoped(
        functools.partial(_body, hbm, vmem, out_copy),
        pltpu.SemaphoreType.DMA((vmem[0].shape[0],)),
        pltpu.SemaphoreType.DMA((7,)))
    out_copy.wait()


def _build(chunk=1024, nbuf=7):
    def call(A_x, A_k_cache, A_v_cache, A_wq, A_wo, B_x, B_w_r, B_w_gate, B_w_up, B_w_down):
        del B_x
        nb, nh, sk, dh = A_k_cache.shape
        split = lambda a, *lead: a.reshape(*lead, -1, a.shape[-1])
        walk = (nb * nh // _PAIR, _PAIR, _RUNS, _TOP, -1, _SUB, dh)
        x = A_x.reshape(nb, A_x.shape[-1])
        weights = (split(A_wq, 2, _WRUNS), split(A_wo, 2, _WRUNS), B_w_r.reshape(-1, 128),
                   split(B_w_gate, 2), split(B_w_up, 2), split(B_w_down, _WRUNS, 2))
        vm = lambda a: pltpu.VMEM(a.shape, a.dtype)
        depth = chunk // (_TOP * _RUNS * _SUB)
        hbm = pl.BlockSpec(memory_space=pltpu.HBM)
        return pl.pallas_call(
            _kernel,
            in_specs=[hbm] * 9,
            out_specs=hbm,
            out_shape=jax.ShapeDtypeStruct(x.shape, x.dtype),
            scratch_shapes=[
                pltpu.VMEM((nbuf, 2, _PAIR, depth, _TOP, _RUNS, _SUB, dh), A_k_cache.dtype),
                vm(x), *map(vm, weights),
                pltpu.VMEM((sk // chunk, _PAIR, _ROWS, chunk), _F32), vm(x),
                pltpu.SemaphoreType.DMA(()),
            ],
            compiler_params=pltpu.CompilerParams(vmem_limit_bytes=64 * 2**20),
        )(x, A_k_cache.reshape(walk), A_v_cache.reshape(walk), *weights).reshape(A_x.shape)

    return call


@jax.jit
def pallas_recurrent_scan__mha_block_cached__moe_arch_mod__decode_kernel(
    A_x: jax.Array,
    A_k_cache: jax.Array,
    A_v_cache: jax.Array,
    A_wq: jax.Array,
    A_wo: jax.Array,
    B_x: jax.Array,
    B_w_r: jax.Array,
    B_w_gate: jax.Array,
    B_w_up: jax.Array,
    B_w_down: jax.Array,
):
    return _build()(A_x, A_k_cache, A_v_cache, A_wq, A_wo, B_x, B_w_r, B_w_gate, B_w_up, B_w_down)
```
